```python
import os as _os
_os.environ.setdefault("JAX_PLATFORMS", "cpu")
import jax
import jax.numpy as jnp

def _softmax(x, axis=-1):
    return jax.nn.softmax(x, axis=axis)
def _gelu(x):
    return jax.nn.gelu(x, approximate=True)
def _silu(x):
    return jax.nn.silu(x)
def _sigmoid(x):
    return jax.nn.sigmoid(x)
def _layernorm(x, axis=-1, eps=1e-5):
    m = jnp.mean(x, axis=axis, keepdims=True)
    v = jnp.var(x, axis=axis, keepdims=True)
    return (x - m) / jnp.sqrt(v + eps)
def _scatter_add(tgt, idx, src, axis=0):
    return tgt.at[idx].add(src)
def _segment_sum(src, seg, n):
    return jax.ops.segment_sum(src, seg, n)
class _Rng:
    def __init__(self, key):
        self._k = key
    def _next(self):
        self._k, sub = jax.random.split(self._k)
        return sub
    def normal(self, shape):
        return jax.random.normal(self._next(), shape, dtype=jnp.bfloat16)
    def randint(self, lo, hi, shape):
        return jax.random.randint(self._next(), shape, lo, hi, dtype=jnp.int32)
    def uniform(self, shape, lo=0.0, hi=1.0):
        return jax.random.uniform(self._next(), shape, jnp.bfloat16, lo, hi)
    def permutation(self, n):
        return jax.random.permutation(self._next(), n)


kernel_name = 'interleave_layers__softmax_full_mha__glu_gated_bilinear__prompt'

def setup_inputs():
    _rng = _Rng(jax.random.key(int.from_bytes(__import__("os").urandom(4), "little")))
    _w = (lambda a: (lambda t: t.astype(jnp.bfloat16) if jnp.issubdtype(t.dtype, jnp.floating) else t)(jnp.asarray(a)))
    def _A_setup():
        B, S, D = 1, 2048, 512
        return {
            "x": _w((lambda *s: _rng.normal(s) * 0.05)(B, S, D)),
            "wqkv": _w((lambda *s: _rng.normal(s) * 0.05)(D, 3 * D)),
            "wo": _w((lambda *s: _rng.normal(s) * 0.05)(D, D)),
        }
    _A_in = _A_setup()

    def _B_setup():
        B, S, D, F = 1, 2048, 512, 1792
        return {
            "x": _w((lambda *s: _rng.normal(s) * 0.05)(B, S, D)),
            "w_gate": _w((lambda *s: _rng.normal(s) * 0.4)(D, F) * (D ** -0.5)),
            "w_up": _w((lambda *s: _rng.normal(s) * 0.4)(D, F) * (D ** -0.5)),
            "w_down": _w((lambda *s: _rng.normal(s) * 0.4)(F, D) * (F ** -0.5)),
        }
    _B_in = _B_setup()

    return {
        "A_x": _A_in["x"],
        "A_wqkv": _A_in["wqkv"],
        "A_wo": _A_in["wo"],
        "B_x": _B_in["x"],
        "B_w_gate": _B_in["w_gate"],
        "B_w_up": _B_in["w_up"],
        "B_w_down": _B_in["w_down"],
    }

def reference(A_x, A_wqkv, A_wo, B_x, B_w_gate, B_w_up, B_w_down):
    def _A_ref(x, wqkv, wo):
        B, S, D = x.shape
        H = 32; Dh = D // H
        qkv = (lambda x, *d: x.transpose(*d))((x @ wqkv).reshape(B, S, 3, H, Dh), 2, 0, 3, 1, 4)
        q, k, v = qkv[0], qkv[1], qkv[2]
        scale = Dh ** -0.5
        scores = jnp.einsum("bhqd,bhkd->bhqk", q, k) * scale
        p = _softmax(scores, axis=-1)
        o = jnp.einsum("bhqk,bhkd->bhqd", p, v)
        return (lambda x, *d: x.transpose(*d))(o, 0, 2, 1, 3).reshape(B, S, D) @ wo

    def _B_ref(x, w_gate, w_up, w_down):
        g = jnp.einsum("bsd,df->bsf", x, w_gate)
        u = jnp.einsum("bsd,df->bsf", x, w_up)
        h = g * u
        return jnp.einsum("bsf,fd->bsd", h, w_down)

    x = A_x
    x = x + _A_ref(_layernorm(x, axis=-1), A_wqkv, A_wo)
    x = x + _B_ref(_layernorm(x, axis=-1), B_w_gate, B_w_up, B_w_down)
    x = x + _A_ref(_layernorm(x, axis=-1), A_wqkv, A_wo)
    x = x + _B_ref(_layernorm(x, axis=-1), B_w_gate, B_w_up, B_w_down)
    return x
```

```python
import functools
import jax
import jax.numpy as jnp
from jax import lax
import jax.experimental.pallas as pl
import jax.experimental.pallas.tpu as pltpu

S, D, H, DH, F = 2048, 512, 32, 16, 1792
TQ = 512
TK = 128
TM = 512
NQ = S // TQ
NC = S // TK
NIT = H * NQ
NM = S // TM
EPS = 1e-5
QSCALE = (DH ** -0.5) * 1.4426950408889634
BF = jnp.bfloat16
F32 = jnp.float32


def _ln(x):
    m = jnp.mean(x, axis=-1, keepdims=True)
    xc = x - m
    v = jnp.mean(xc * xc, axis=-1, keepdims=True)
    return xc * lax.rsqrt(v + EPS)


def _kernel(x_hbm, wqkv_hbm, wo_hbm, wg_hbm, wu_hbm, wd_hbm, out_hbm,
            xio, wqkv, wo, wg, wu, wd, wqvt, xres, ks, qts, vts, ots, ss, sems):
    cp_x = pltpu.make_async_copy(x_hbm, xio, sems.at[0])
    cp_qkv = pltpu.make_async_copy(wqkv_hbm, wqkv, sems.at[1])
    cp_wo = pltpu.make_async_copy(wo_hbm, wo, sems.at[2])
    cp_wg = pltpu.make_async_copy(wg_hbm, wg, sems.at[3])
    cp_wu = pltpu.make_async_copy(wu_hbm, wu, sems.at[4])
    cp_wd = pltpu.make_async_copy(wd_hbm, wd, sems.at[5])
    cp_qkv.start(); cp_x.start()
    cp_wo.start(); cp_wg.start(); cp_wu.start(); cp_wd.start()
    cp_qkv.wait()
    wqvt[0:D, :] = wqkv[:, 0:D].astype(F32).T.astype(BF)
    wqvt[D:2 * D, :] = wqkv[:, 2 * D:3 * D].astype(F32).T.astype(BF)
    cp_x.wait()

    def qkv_block(i, x):
        xn = _ln(x).astype(BF)
        k = jnp.dot(xn, wqkv[:, D:2 * D], preferred_element_type=F32).astype(BF)
        r0 = pl.multiple_of(i * TM, TM)
        for g in range(4):
            ks[g, pl.ds(r0, TM), :] = k[:, g * 128:(g + 1) * 128]
        qv = lax.dot_general(wqvt[...], xn, (((1,), (1,)), ((), ())), preferred_element_type=F32)
        qts[i] = (qv[0:D] * QSCALE).astype(BF)
        vts[i] = qv[D:2 * D].astype(BF)

    def first_block(i, _):
        r0 = pl.multiple_of(i * TM, TM)
        x = xio[pl.ds(r0, TM), :].astype(F32)
        xres[pl.ds(r0, TM), :] = x
        qkv_block(i, x)
        return 0
    lax.fori_loop(0, NM, first_block, 0)

    def red(x, op):
        return op(x.reshape(TK // 8, 8, TQ), axis=0)

    def get_w(it):
        h = lax.shift_right_logical(it, 2)
        qb = it & 3
        g = lax.shift_right_logical(h, 3)
        hh = h & 7
        qg = qts[qb, pl.ds(pl.multiple_of(g * 128, 128), 128), :]
        row = lax.broadcasted_iota(jnp.int32, (128, TQ), 0)
        w = jnp.where(lax.shift_right_logical(row, 4) == hh, qg, jnp.zeros_like(qg))
        return w, g

    def a_chunk(w, g, c):
        return jnp.dot(ks[g, c * TK:(c + 1) * TK, :], w, preferred_element_type=F32)

    def attention():
        w, g = get_w(jnp.int32(0))
        m = jnp.full((8, TQ), -jnp.inf, F32)
        for c in range(NC):
            s = a_chunk(w, g, c)
            ss[c] = s
            m = jnp.maximum(m, red(s, jnp.max))
        m = jnp.max(m, axis=0, keepdims=True)

        def body(it, m_cur):
            h = lax.shift_right_logical(it, 2)
            qb = it & 3
            h0 = pl.multiple_of(h * DH, DH)
            nxt = jnp.minimum(it + 1, NIT - 1)
            w, g = get_w(nxt)
            m_next = jnp.full((8, TQ), -jnp.inf, F32)
            l = jnp.zeros((8, TQ), F32)
            acc = jnp.zeros((DH, TQ), F32)
            for c in range(NC):
                s_new = a_chunk(w, g, c)
                p = jnp.exp2(ss[c] - m_cur)
                l = l + red(p, jnp.sum)
                kb, ko = (c * TK) // TM, (c * TK) % TM
                acc = acc + jnp.dot(vts[kb, pl.ds(h0, DH), ko:ko + TK], p.astype(BF),
                                    preferred_element_type=F32)
                ss[c] = s_new
                m_next = jnp.maximum(m_next, red(s_new, jnp.max))
            l = jnp.sum(l, axis=0, keepdims=True)
            ots[qb, pl.ds(h0, DH), :] = (acc / l).astype(BF)
            return jnp.max(m_next, axis=0, keepdims=True)
        lax.fori_loop(0, NIT, body, m)

    def post_block(i):
        r0 = pl.multiple_of(i * TM, TM)
        attn = lax.dot_general(ots[i], wo[...], (((0,), (0,)), ((), ())), preferred_element_type=F32)
        x1 = xres[pl.ds(r0, TM), :] + attn
        xn = _ln(x1).astype(BF)
        gt = jnp.dot(xn, wg[...], preferred_element_type=F32)
        up = jnp.dot(xn, wu[...], preferred_element_type=F32)
        hh = (gt * up).astype(BF)
        y = jnp.dot(hh, wd[...], preferred_element_type=F32)
        return x1 + y

    attention()
    cp_wo.wait(); cp_wg.wait(); cp_wu.wait(); cp_wd.wait()

    def mid_block(i, _):
        r0 = pl.multiple_of(i * TM, TM)
        x2 = post_block(i)
        xres[pl.ds(r0, TM), :] = x2
        qkv_block(i, x2)
        return 0
    lax.fori_loop(0, NM, mid_block, 0)

    attention()

    def out_copy(i):
        r0 = pl.multiple_of(i * TM, TM)
        return pltpu.make_async_copy(xio.at[pl.ds(r0, TM), :], out_hbm.at[pl.ds(r0, TM), :], sems.at[6 + i])

    def last_block(i, _):
        r0 = pl.multiple_of(i * TM, TM)
        x2 = post_block(i)
        xio[pl.ds(r0, TM), :] = x2.astype(BF)
        out_copy(i).start()
        return 0
    lax.fori_loop(0, NM, last_block, 0)
    for i in range(NM):
        out_copy(i).wait()


@jax.jit
def pallas_interleave_layers__softmax_full_mha__glu_gated_bilinear__prompt_kernel(
        A_x, A_wqkv, A_wo, B_x, B_w_gate, B_w_up, B_w_down):
    x = A_x.reshape(S, D)
    out = pl.pallas_call(
        _kernel,
        out_shape=jax.ShapeDtypeStruct((S, D), BF),
        in_specs=[pl.BlockSpec(memory_space=pl.ANY)] * 6,
        out_specs=pl.BlockSpec(memory_space=pl.ANY),
        scratch_shapes=[
            pltpu.VMEM((S, D), BF),
            pltpu.VMEM((D, 3 * D), BF),
            pltpu.VMEM((D, D), BF),
            pltpu.VMEM((D, F), BF),
            pltpu.VMEM((D, F), BF),
            pltpu.VMEM((F, D), BF),
            pltpu.VMEM((2 * D, D), BF),
            pltpu.VMEM((S, D), F32),
            pltpu.VMEM((4, S, 128), BF),
            pltpu.VMEM((NQ, D, TQ), BF),
            pltpu.VMEM((NM, D, TM), BF),
            pltpu.VMEM((NQ, D, TQ), BF),
            pltpu.VMEM((NC, TK, TQ), F32),
            pltpu.SemaphoreType.DMA((6 + NM,)),
        ],
        compiler_params=pltpu.CompilerParams(vmem_limit_bytes=100 * 1024 * 1024),
    )(x, A_wqkv, A_wo, B_w_gate, B_w_up, B_w_down)
    return out.reshape(1, S, D)
```

```python
import jax
import jax.numpy as jnp
from jax import lax
import jax.experimental.pallas as pl
import jax.experimental.pallas.tpu as pltpu

S, D, H, DH, F = 2048, 512, 32, 16, 1792
TQ = 512
TK = 128
TM = 512
NQ = S // TQ
NC = S // TK
NJ = TQ // 128
NM = S // TM
RV = 16
NKV = RV * NC
LAG = 3
NS = 4
HB = 1
NSTEP = NQ * NC * HB
EPS = 1e-5
QSCALE = (DH ** -0.5) * 1.4426950408889634
L_LO = 2.0 ** -30
L_HI = 2.0 ** 60
BF = jnp.bfloat16
F32 = jnp.float32
U32 = jnp.uint32
FORCE_SLOW = False
NSUB = 2
NSUB0 = 2


def _ln(x):
    m = jnp.mean(x, axis=-1, keepdims=True)
    xc = x - m
    v = jnp.mean(xc * xc, axis=-1, keepdims=True)
    return xc * lax.rsqrt(v + EPS)


def _packi(x):
    n = x.shape[0] // 16
    a = jnp.concatenate([x[j * 16:j * 16 + 8] for j in range(n)], axis=0) if n > 1 else x[0:8]
    b = jnp.concatenate([x[j * 16 + 8:j * 16 + 16] for j in range(n)], axis=0) if n > 1 else x[8:16]
    return pltpu.pack_elementwise([a, b], packed_dtype=BF)


def _rowsum8(l, x):
    for r in range(x.shape[0] // 8):
        l = l + x[r * 8:(r + 1) * 8]
    return l


def _kernel(x_hbm, wqkv_hbm, wo_hbm, wg_hbm, wu_hbm, wd_hbm, out_hbm,
            xio, wqkv, wo, wg, wu, wd, wqvt, xres, kr, qtu, qf, vtu, ots, pring, kba, kbb, ss, sems):
    def x_copy(i):
        r0 = pl.multiple_of(i * TM, TM)
        return pltpu.make_async_copy(x_hbm.at[pl.ds(r0, TM), :], xio.at[pl.ds(r0, TM), :], sems.at[6 + i])

    cp_qkv = pltpu.make_async_copy(wqkv_hbm, wqkv, sems.at[1])
    cp_wo = pltpu.make_async_copy(wo_hbm, wo, sems.at[2])
    cp_wg = pltpu.make_async_copy(wg_hbm, wg, sems.at[3])
    cp_wu = pltpu.make_async_copy(wu_hbm, wu, sems.at[4])
    cp_wd = pltpu.make_async_copy(wd_hbm, wd, sems.at[5])
    cp_qkv.start()
    x_copy(0).start()
    with jax.named_scope('w0'):
        cp_qkv.wait()
    for i in range(1, NM):
        x_copy(i).start()
    wqvt[0:D, :] = wqkv[:, 0:D].astype(F32).T.astype(BF)
    wqvt[D:2 * D, :] = wqkv[:, 2 * D:3 * D].astype(F32).T.astype(BF)

    nt = (((1,), (1,)), ((), ()))

    def qkv_part(i, u, n, x):
        xn = _ln(x)
        xnb = xn.astype(BF)
        xni = pltpu.bitcast(_packi(xn), BF)
        k = jnp.dot(xnb, wqkv[:, D:2 * D], preferred_element_type=F32)
        ku = pltpu.bitcast(k.astype(BF), U32)
        rk = pl.multiple_of(i * (TM // 2) + u * (n // 2), n // 2)
        for h in range(H):
            g, hh = divmod(h, 8)
            kg = ku[:, g * 128:(g + 1) * 128]
            kr[h, pl.ds(rk, n // 2), :] = pltpu.roll(kg, 128 - 16 * hh, 1) if hh else kg
        qt = lax.dot_general(wqvt[0:D, :], xnb, nt, preferred_element_type=F32) * QSCALE
        qb16 = qt.astype(BF)
        qtu[:, i, :, u * n:(u + 1) * n] = pltpu.bitcast(qb16, U32).reshape(H, 8, n)
        q32 = qb16.astype(F32)
        for j in range(n // 128):
            qf[:, i, u * (n // 128) + j] = q32[:, j * 128:(j + 1) * 128].reshape(H, DH, 128)
        vt = lax.dot_general(wqvt[D:2 * D, :], xni, nt, preferred_element_type=F32)
        vtu[:, i, :, u * n:(u + 1) * n] = pltpu.bitcast(vt.astype(BF), U32).reshape(H, 8, n)

    def first_block(i, _):
        x_copy(i).wait()
        n = TM // NSUB0
        for u in range(NSUB0):
            r0 = pl.multiple_of(i * TM + u * n, n)
            x = xio[pl.ds(r0, n), :].astype(F32)
            xres[pl.ds(r0, n), :] = x
            qkv_part(i, u, n, x)
        return 0

    def get_w(h, qb):
        q = pltpu.bitcast(qtu[h, qb], BF)
        return jnp.concatenate([q, jnp.zeros((128 - DH, TQ), BF)], axis=0)

    def get_v(h, c):
        kb_, ko = divmod(c * TK, TM)
        return pltpu.bitcast(vtu[h, kb_, :, ko:ko + TK], BF)

    def kb_make(h, kb_ref, hh):
        ku = jnp.concatenate([kr[h, c * (TK // 2):c * (TK // 2) + RV // 2, :] for c in range(NC)], axis=0)
        kf = pltpu.bitcast(ku, BF).astype(F32)
        for d in range(DH):
            kb_ref[hh * DH + d] = jnp.broadcast_to(kf[:, d:d + 1], (NKV, 128))

    def vpu_block(h, kb_ref, hh, qb, r0, j, z, anc):
        acc = None
        for d in range(DH):
            kb = kb_ref[z + (hh * DH + d), r0:r0 + 16, :]
            q = qf[h + z, qb, j, pl.ds(d, 8, stride=0), :]
            if d == 0:
                q = jnp.maximum(q, jnp.minimum(q, anc))
            t = kb * jnp.concatenate([q, q], axis=0)
            acc = t if acc is None else acc + t
        return jnp.exp2(acc)

    def ab_step(w, h, kb_ref, hh, qb, c, slot, l, lv, zs, prev):
        r = RV if kb_ref is not None else 0
        s = jnp.dot(pltpu.bitcast(kr[h, (c * TK + r) // 2:(c + 1) * TK // 2, :], BF), w,
                    preferred_element_type=F32)
        p = jnp.exp2(s)
        l = _rowsum8(l, p)
        pring[slot, r // 2:, :] = _packi(p)
        if r:
            pa = p if prev is None else prev
            na = pa.shape[0] // 8
            lv = list(lv)
            for j in range(NJ):
                ia = (j * na) // NJ
                pv = vpu_block(h, kb_ref, hh, qb, c * RV, j, zs[j], pa[ia * 8:(ia + 1) * 8, j * 128:(j + 1) * 128])
                lv[j] = pv[0:8] + pv[8:16] if lv[j] is None else lv[j] + pv[0:8] + pv[8:16]
                pring[slot, 0:8, j * 128:(j + 1) * 128] = _packi(pv)
        return l, lv, p

    zero = jnp.zeros((8, TQ), F32)

    def region(it, carry, kb_r, kb_w):
        l_part, bad = carry
        h0 = it * HB
        zs = [lax.shift_right_logical(it + j, 16) for j in range(NJ)]
        for hh in range(HB):
            kb_make(jnp.minimum(h0 + HB + hh, H - 1), kb_w, hh)
        w = None
        acc = None
        prev = None
        lv = [None] * NJ
        for t in range(NSTEP):
            hh, s_ = divmod(t, NQ * NC)
            qb, c = divmod(s_, NC)
            ta = t + LAG
            ahead = ta >= NSTEP
            ha, sa = divmod(ta, NQ * NC)
            qa, ca = divmod(sa, NC)
            h_a = jnp.minimum(h0 + ha, H - 1) if ahead else h0 + ha
            if ca == 0 or w is None:
                w = get_w(h_a, qa)
            if c == 0:
                if acc is None:
                    l2 = jnp.concatenate([carry[0], carry[0]], axis=0)
                    acc = jnp.where(l2 < 0, l2, 0.0)
                else:
                    acc = jnp.where(acc > jnp.inf, acc, 0.0)
            p = pltpu.bitcast(pring[t % NS], BF)
            l_part, lv, prev = ab_step(w, h_a, None if ahead else kb_r, ha, qa, ca, ta % NS, l_part, lv, zs, prev)
            acc = acc + jnp.dot(get_v(h0 + hh, c), p, preferred_element_type=F32)
            if ca == NC - 1:
                l_done = l_part + jnp.concatenate(lv, axis=1)
                l_part = zero
                lv = [None] * NJ
            if c == NC - 1:
                lt = jnp.sum(l_done, axis=0, keepdims=True)
                ok = jnp.logical_and(lt > L_LO, lt < L_HI)
                big = jnp.maximum(jnp.abs(acc[0:8]), jnp.abs(acc[8:16]))
                ok = jnp.logical_and(ok, big < jnp.inf)
                bad = jnp.maximum(bad, jnp.where(ok, 0.0, 1.0))
                ots[qb, pl.ds(pl.multiple_of((h0 + hh) * DH, DH), DH), :] = (acc / lt).astype(BF)
        return l_part, bad

    def attention_fast():
        for hh in range(HB):
            kb_make(hh, kba, hh)
        l_part = zero
        w = get_w(0, 0)
        for t in range(LAG):
            l_part, _, _ = ab_step(w, 0, None, 0, 0, t, t % NS, l_part, None, None, None)

        def body(it, carry):
            return lax.cond((it & 1) == 0,
                            lambda cr: region(it, cr, kba, kbb),
                            lambda cr: region(it, cr, kbb, kba), carry)
        _, bad = lax.fori_loop(0, H // HB, body, (l_part, zero))
        return jnp.max(bad)

    def attention_exact():
        def unit(u, _):
            h = lax.shift_right_logical(u, 2)
            qb = u & (NQ - 1)
            w = get_w(h, qb)
            m = jnp.full((8, TQ), -jnp.inf, F32)
            for c in range(NC):
                s = jnp.dot(pltpu.bitcast(kr[h, c * TK // 2:(c + 1) * TK // 2, :], BF), w,
                            preferred_element_type=F32)
                ss[c] = s
                for r in range(TK // 8):
                    m = jnp.maximum(m, s[r * 8:(r + 1) * 8])
            m = jnp.max(m, axis=0, keepdims=True)
            l = zero
            acc = jnp.zeros((DH, TQ), F32)
            for c in range(NC):
                p = jnp.exp2(ss[c] - m)
                l = _rowsum8(l, p)
                acc = acc + jnp.dot(get_v(h, c), pltpu.bitcast(_packi(p), BF), preferred_element_type=F32)
            lt = jnp.sum(l, axis=0, keepdims=True)
            ots[qb, pl.ds(pl.multiple_of(h * DH, DH), DH), :] = (acc / lt).astype(BF)
            return 0
        lax.fori_loop(0, H * NQ, unit, 0)

    def out_copy(i):
        r0 = pl.multiple_of(i * TM, TM)
        return pltpu.make_async_copy(xio.at[pl.ds(r0, TM), :], out_hbm.at[pl.ds(r0, TM), :], sems.at[6 + i])

    def post_parts(i, n):
        us = range(TM // n)
        rows = [pl.ds(pl.multiple_of(i * TM + u * n, n), n) for u in us]
        x1 = [xres[rows[u], :] + lax.dot_general(ots[i, :, u * n:(u + 1) * n], wo[...], (((0,), (0,)), ((), ())),
                                                 preferred_element_type=F32) for u in us]
        xn = [_ln(x1[u]).astype(BF) for u in us]
        hh = [(jnp.dot(xn[u], wg[...], preferred_element_type=F32)
               * jnp.dot(xn[u], wu[...], preferred_element_type=F32)).astype(BF) for u in us]
        return rows, [x1[u] + jnp.dot(hh[u], wd[...], preferred_element_type=F32) for u in us]

    def mid_block(i, _):
        n = TM // NSUB
        rows, xs = post_parts(i, n)
        for u in range(NSUB):
            xres[rows[u], :] = xs[u]
            qkv_part(i, u, n, xs[u])
        return 0

    def last_block(i, _):
        rows, xs = post_parts(i, TM // NSUB)
        for u in range(NSUB):
            xio[rows[u], :] = xs[u].astype(BF)
        out_copy(i).start()
        return 0

    with jax.named_scope('first'):
        lax.fori_loop(0, NM, first_block, 0)
    cp_wo.start(); cp_wg.start(); cp_wu.start(); cp_wd.start()

    for li in range(2):
        with jax.named_scope('attn'):
            bad = attention_fast()

        @pl.when((bad > 0.0) if not FORCE_SLOW else (bad > -1.0))
        def _():
            attention_exact()

        if li == 0:
            cp_wo.wait(); cp_wg.wait(); cp_wu.wait(); cp_wd.wait()
            with jax.named_scope('mid'):
                lax.fori_loop(0, NM, mid_block, 0)
        else:
            with jax.named_scope('last'):
                lax.fori_loop(0, NM, last_block, 0)

    with jax.named_scope('w2'):
        for i in range(NM):
            out_copy(i).wait()


@jax.jit
def pallas_interleave_layers__softmax_full_mha__glu_gated_bilinear__prompt_kernel(
        A_x, A_wqkv, A_wo, B_x, B_w_gate, B_w_up, B_w_down):
    x = A_x.reshape(S, D)
    out = pl.pallas_call(
        _kernel,
        out_shape=jax.ShapeDtypeStruct((S, D), BF),
        in_specs=[pl.BlockSpec(memory_space=pl.ANY)] * 6,
        out_specs=pl.BlockSpec(memory_space=pl.ANY),
        scratch_shapes=[
            pltpu.VMEM((S, D), BF),
            pltpu.VMEM((D, 3 * D), BF),
            pltpu.VMEM((D, D), BF),
            pltpu.VMEM((D, F), BF),
            pltpu.VMEM((D, F), BF),
            pltpu.VMEM((F, D), BF),
            pltpu.VMEM((2 * D, D), BF),
            pltpu.VMEM((S, D), F32),
            pltpu.VMEM((H, S // 2, 128), U32),
            pltpu.VMEM((H, NQ, 8, TQ), U32),
            pltpu.VMEM((H, NQ, NJ, DH, 128), F32),
            pltpu.VMEM((H, NM, 8, TM), U32),
            pltpu.VMEM((NQ, D, TQ), BF),
            pltpu.VMEM((NS, TK // 2, TQ), U32),
            pltpu.VMEM((HB * DH, NKV, 128), F32),
            pltpu.VMEM((HB * DH, NKV, 128), F32),
            pltpu.VMEM((NC, TK, TQ), F32),
            pltpu.SemaphoreType.DMA((6 + NM,)),
        ],
        compiler_params=pltpu.CompilerParams(vmem_limit_bytes=100 * 1024 * 1024),
    )(x, A_wqkv, A_wo, B_w_gate, B_w_up, B_w_down)
    return out.reshape(1, S, D)
```

```python
import jax
import jax.numpy as jnp
from jax import lax
import jax.experimental.pallas as pl
import jax.experimental.pallas.tpu as pltpu

S, D, H, DH, F = 2048, 512, 32, 16, 1792
TQ = 512
TK = 128
TM = 512
TN = 128
NQ = S // TQ
NC = S // TK
NJ = TQ // 128
NM = S // TM
NU = TM // TN
NSTEP = NQ * NC
EPS = 1e-5
QSCALE = (DH ** -0.5) * 1.4426950408889634
L_LO = 2.0 ** -30
L_HI = 2.0 ** 60
V_HI = 2.0 ** 60
BF = jnp.bfloat16
F32 = jnp.float32
U32 = jnp.uint32

NPRE = 8
V0 = 2
AOFF = -6
MX = [(g, i) for g in range(NSTEP + 2) for i in range(7, -1 if g % NSTEP < V0 else 0, -1)]
NMX = 7 * NSTEP + V0
LAST = {g: n for n, (g, _) in enumerate(MX)}
SUB = 4
P0, PN, FREE = 1, 60, 4
PLIST = [(k, idx, sub) for idx in range(16) for sub in range(SUB) for k in (0, 1)]


def _ln(x):
    m = jnp.mean(x, axis=-1, keepdims=True)
    xc = x - m
    v = jnp.mean(xc * xc, axis=-1, keepdims=True)
    return (xc * lax.rsqrt(v + EPS)).astype(BF)


def _swap8(x):
    return jnp.concatenate([x[r ^ 8:(r ^ 8) + 8] for r in range(0, x.shape[0], 8)], axis=0)


def _rowsum8(l, x):
    y = jnp.sum(x.reshape(x.shape[0] // 8, 8, x.shape[1]), axis=0)
    return y if l is None else l + y


def _kernel(x_hbm, wqkv_hbm, wo_hbm, wg_hbm, wu_hbm, wd_hbm, out_hbm,
            xio, wq, wk, wv, wo, wg, wu, wd, wqvt, xres, kr, qtu, vts, ots,
            ppre, kba, kbb, qba, qbb, ss, lts, vmx, sems):
    parts = range(NU)
    nt = (((1,), (1,)), ((), ()))

    def rows_of(i, u):
        return pl.ds(pl.multiple_of(i * TM + u * TN, TN), TN)

    def x_copy(i):
        return pltpu.make_async_copy(x_hbm.at[i * TM:(i + 1) * TM, :], xio.at[i * TM:(i + 1) * TM, :],
                                     sems.at[(0, 3, 6, 6)[i]])

    def out_copy(i, u):
        return pltpu.make_async_copy(xio.at[rows_of(i, u), :], out_hbm.at[rows_of(i, u), :], sems.at[5])

    cp_wk = pltpu.make_async_copy(wqkv_hbm.at[:, D:2 * D], wk, sems.at[1])
    cp_wq = pltpu.make_async_copy(wqkv_hbm.at[:, 0:D], wq, sems.at[2])
    cp_wv = pltpu.make_async_copy(wqkv_hbm.at[:, 2 * D:3 * D], wv, sems.at[3])
    cp_late = [pltpu.make_async_copy(src, dst, sems.at[4])
               for src, dst in ((wo_hbm, wo), (wg_hbm, wg), (wu_hbm, wu), (wd_hbm, wd))]

    def k_mm(xn):
        k = jnp.dot(xn, wk[...], preferred_element_type=F32)
        return pltpu.bitcast(_swap8(k).astype(BF), U32)

    def k_store(i, u, ku):
        rk = pl.ds(pl.multiple_of((i * NU + u) * (TN // 2), TN // 2), TN // 2)
        for h in range(H):
            g, hh = divmod(h, 8)
            kg = ku[:, g * 128:(g + 1) * 128]
            kr[h, rk, :] = pltpu.roll(kg, 128 - 16 * hh, 1) if hh else kg
        kf = pltpu.bitcast(ku[0:8, 0:128], BF).astype(F32)
        rb = pl.ds(pl.multiple_of((i * NU + u) * 16, 16), 16)
        for d in range(DH):
            kba[0, d, rb, :] = jnp.broadcast_to(kf[:, d:d + 1], (16, 128))

    def q_store(i, u, qt):
        q16 = (qt * QSCALE).astype(BF)
        qtu[:, i, :, u * TN:(u + 1) * TN] = pltpu.bitcast(q16, U32).reshape(H, 8, TN)
        q0 = q16[0:DH].astype(F32)
        for d in range(DH):
            qba[0, i, u, d] = jnp.broadcast_to(q0[d:d + 1, :], (8, 128))

    def v_store(i, u, vt):
        vts[:, i, :, u * TN:(u + 1) * TN] = vt.reshape(H, DH, TN)
        vmx[i, :, u * TN:(u + 1) * TN] = jnp.max(jnp.abs(vt).reshape(D // 8, 8, TN), axis=0)

    def qkv_part(i, u, xn):
        k_store(i, u, k_mm(xn))
        qv = lax.dot_general(wqvt[...], xn, nt, preferred_element_type=F32)
        q_store(i, u, qv[0:D])
        v_store(i, u, qv[D:2 * D])

    def load_ln(i, u):
        x = xio[rows_of(i, u), :].astype(F32)
        xres[rows_of(i, u), :] = x
        return _ln(x)

    def first_phase():
        x_copy(0).start()
        cp_wk.start()
        cp_wq.start()
        cp_wv.start()
        for i in range(1, NM):
            x_copy(i).start()
        x_copy(0).wait()
        xn = [load_ln(0, u) for u in parts]
        cp_wk.wait()
        kus = [k_mm(xn[u]) for u in parts[:NU // 2]]
        cp_wq.wait()
        kus += [k_mm(xn[u]) for u in parts[NU // 2:]]
        for u in parts:
            k_store(0, u, kus[u])
        wqt = wq[...].astype(F32).T.astype(BF)
        wqvt[0:D, :] = wqt
        for u in parts:
            q_store(0, u, lax.dot_general(wqt, xn[u], nt, preferred_element_type=F32))
        cp_wv.wait()
        x_copy(1).wait()
        wvt = wv[...].astype(F32).T.astype(BF)
        wqvt[D:2 * D, :] = wvt
        for u in parts:
            v_store(0, u, lax.dot_general(wvt, xn[u], nt, preferred_element_type=F32))
        xn_next = load_ln(1, 0)
        for i in range(2, NM):
            x_copy(i).wait()
        for cp in cp_late:
            cp.start()

        def block(i, xn0):
            for u in parts:
                qkv_part(i, u, xn0 if u == 0 else load_ln(i, u))
            return load_ln(jnp.minimum(i + 1, NM - 1), 0)
        lax.fori_loop(1, NM, block, xn_next)

    def get_w(h, qb):
        return jnp.concatenate([pltpu.bitcast(qtu[h, qb], BF), jnp.zeros((128 - DH, TQ), BF)], axis=0)

    def a_dot(h, w, tiles):
        ku = jnp.concatenate([kr[h, c * 64 + i * 8:c * 64 + (i + 1) * 8, :] for c, i in tiles], axis=0)
        return jnp.exp2(jnp.dot(pltpu.bitcast(ku, BF), w, preferred_element_type=F32))

    def prep_piece(h, bufs, i, anc):
        kb_ref, qb_ref = bufs
        kind, idx, sub = PLIST[i]
        qb, j = divmod(idx, NJ)
        src = kr[h, idx * 64:idx * 64 + 8, :] if kind == 0 else qtu[h, qb, :, j * 128:(j + 1) * 128]
        if anc is not None:
            src = jnp.where(anc < 0, jnp.uint32(0), src)
        val = pltpu.bitcast(src, BF).astype(F32)
        for d in range(sub * (DH // SUB), (sub + 1) * (DH // SUB)):
            if kind == 0:
                kb_ref[0, d, idx * 16:(idx + 1) * 16, :] = jnp.broadcast_to(val[:, d:d + 1], (16, 128))
            else:
                qb_ref[0, qb, j, d] = jnp.broadcast_to(val[d:d + 1, :], (8, 128))

    def vpu_block(bufs, qb, c, j, z, anc):
        kb_ref, qb_ref = bufs
        kb = kb_ref[z, :, c * 16:(c + 1) * 16, :].reshape(DH, 2, 8, 128)
        q = qb_ref[z, qb, j]
        q0 = jnp.maximum(q[0], jnp.minimum(q[0], anc))
        q = jnp.concatenate([q0[None], q[1:]], axis=0)
        return jnp.exp2(jnp.sum(kb * q[:, None], axis=0).reshape(16, 128))

    def head(h, l_in, rd, wr):
        zs = [lax.shift_right_logical(h + j, 16) for j in range(2 * NJ)]
        hn = jnp.minimum(h + 1, H - 1)
        pt = {MX[n]: ppre[n] for n in range(NPRE)}
        ls = {0: l_in}
        ws = {}
        hist = {}
        acc = None
        nxt, ksub, kp = NPRE, V0 * NJ, 0
        for g in range(NSTEP):
            qb, c = divmod(g, NC)
            end = LAST[g] + NPRE + 1
            byunit = {}
            for n in range(nxt, end):
                byunit.setdefault(MX[n][0] // NC, []).append(n)
            nxt = end
            for u, nl in byunit.items():
                hu = hn if u == NQ else h
                if u not in ws:
                    ws[u] = get_w(hu, u % NQ)
                p = a_dot(hu, ws[u], [(MX[n][0] % NC, MX[n][1]) for n in nl])
                ls[u] = _rowsum8(ls.get(u), p)
                for k, n in enumerate(nl):
                    hist[n] = p[k * 16:(k + 1) * 16]
                    if u == NQ:
                        ppre[n - NMX] = hist[n]
                    else:
                        pt[MX[n]] = hist[n]
            while kp < len(PLIST):
                a = NPRE + (P0 * NMX) // NSTEP + (kp * PN * NMX) // (NSTEP * len(PLIST))
                if a >= end:
                    break
                free = PLIST[kp][0] == 1 and PLIST[kp][1] >= 16 - FREE
                prep_piece(hn, wr, kp, None if free else hist[a][8:16, 0:128])
                kp += 1
            while ksub < NSTEP * NJ:
                gv, j = divmod(ksub, NJ)
                a = (ksub * 7) // NJ + V0 + AOFF
                if a >= end:
                    break
                qv, cv = divmod(gv, NC)
                pv = vpu_block(rd, qv, cv, j, zs[ksub % len(zs)], hist[a][0:8, j * 128:(j + 1) * 128])
                ls[('v', qv, j)] = _rowsum8(ls.get(('v', qv, j)), pv)
                pt[(gv, 0, j)] = pv
                ksub += 1
            if c == 0:
                if acc is None:
                    l2 = jnp.concatenate([l_in, l_in], axis=0)
                    acc = jnp.where(l2 < 0, l2, 0.0)
                else:
                    acc = jnp.where(acc > jnp.inf, acc, 0.0)
            if g >= V0:
                pt[(g, 0)] = jnp.concatenate([pt.pop((g, 0, j)) for j in range(NJ)], axis=1)
            p = _swap8(jnp.concatenate([pt.pop((g, i)) for i in range(8)], axis=0))
            v = vts[h, c // NU, :, (c % NU) * TK:(c % NU + 1) * TK]
            acc = acc + jnp.dot(v, p, preferred_element_type=F32)
            if c == NC - 1:
                lv = jnp.concatenate([ls[('v', qb, j)] for j in range(NJ)], axis=1)
                lt = jnp.sum(ls[qb] + lv, axis=0, keepdims=True)
                lts[h, qb:qb + 1, :] = lt
                ots[qb, pl.ds(pl.multiple_of(h * DH, DH), DH), :] = (acc / lt).astype(BF)
        return ls[NQ]

    def attention_fast():
        p = a_dot(0, get_w(0, 0), MX[:NPRE])
        for n in range(NPRE):
            ppre[n] = p[n * 16:(n + 1) * 16]

        def body(h, l):
            return lax.cond((h & 1) == 0,
                            lambda x: head(h, x, (kba, qba), (kbb, qbb)),
                            lambda x: head(h, x, (kbb, qbb), (kba, qba)), l)
        lax.fori_loop(0, H, body, _rowsum8(None, p))
        lt = lts[...]
        bad_l = jnp.where(jnp.logical_and(lt > L_LO, lt < L_HI), 0.0, 1.0)
        bad_v = jnp.where(vmx[...] < V_HI, 0.0, 1.0)
        return jnp.maximum(jnp.max(jnp.max(bad_l, axis=0)), jnp.max(jnp.max(bad_v, axis=0)))

    def attention_exact():
        def unit(u, _):
            h = lax.shift_right_logical(u, 2)
            qb = u & (NQ - 1)
            w = get_w(h, qb)

            def pass1(c, m):
                ku = kr[h, pl.ds(pl.multiple_of(c * 64, 64), 64), :]
                s = jnp.dot(pltpu.bitcast(ku, BF), w, preferred_element_type=F32)
                ss[c] = s
                return jnp.maximum(m, jnp.max(s.reshape(TK // 8, 8, TQ), axis=0))
            m = lax.fori_loop(0, NC, pass1, jnp.full((8, TQ), -jnp.inf, F32))
            m = jnp.max(m, axis=0, keepdims=True)

            def pass2(b, carry):
                l, acc = carry
                for cc in parts:
                    p = jnp.exp2(ss[b * NU + cc] - m)
                    l = _rowsum8(l, p)
                    acc = acc + jnp.dot(vts[h, b, :, cc * TK:(cc + 1) * TK], _swap8(p),
                                        preferred_element_type=F32)
                return l, acc
            l, acc = lax.fori_loop(0, NM, pass2, (jnp.zeros((8, TQ), F32), jnp.zeros((DH, TQ), F32)))
            lt = jnp.sum(l, axis=0, keepdims=True)
            ots[qb, pl.ds(pl.multiple_of(h * DH, DH), DH), :] = (acc / lt).astype(BF)
            return 0
        lax.fori_loop(0, H * NQ, unit, 0)

    def o_part(i, u):
        return ots[i, :, u * TN:(u + 1) * TN].T

    def post(i, o0):
        x1 = [xres[rows_of(i, u), :]
              + jnp.dot(o0 if u == 0 else o_part(i, u), wo[...], preferred_element_type=F32) for u in parts]
        xn = [_ln(x1[u]) for u in parts]
        hh = [(jnp.dot(xn[u], wg[...], preferred_element_type=F32)
               * jnp.dot(xn[u], wu[...], preferred_element_type=F32)).astype(BF) for u in parts]
        return [x1[u] + jnp.dot(hh[u], wd[...], preferred_element_type=F32) for u in parts]

    def mid_block(i, o0):
        xs = post(i, o0)
        for u in parts:
            xres[rows_of(i, u), :] = xs[u]
            qkv_part(i, u, _ln(xs[u]))
        return o_part(jnp.minimum(i + 1, NM - 1), 0)

    def last_block(i, o0):
        xs = post(i, o0)
        o_next = o_part(jnp.minimum(i + 1, NM - 1), 0)
        for u in parts:
            xio[rows_of(i, u), :] = xs[u].astype(BF)
            out_copy(i, u).start()
        return o_next

    def redo(_):
        attention_exact()
        return o_part(0, 0)

    first_phase()
    for layer in range(2):
        bad = attention_fast()
        o0 = lax.cond(bad > 0.0, redo, lambda o: o, o_part(0, 0))
        if layer == 0:
            for cp in cp_late:
                cp.wait()
        lax.fori_loop(0, NM, mid_block if layer == 0 else last_block, o0)
    for i in range(NM):
        for u in parts:
            out_copy(i, u).wait()


@jax.jit
def pallas_interleave_layers__softmax_full_mha__glu_gated_bilinear__prompt_kernel(
        A_x, A_wqkv, A_wo, B_x, B_w_gate, B_w_up, B_w_down):
    out = pl.pallas_call(
        _kernel,
        out_shape=jax.ShapeDtypeStruct((S, D), BF),
        in_specs=[pl.BlockSpec(memory_space=pl.ANY)] * 6,
        out_specs=pl.BlockSpec(memory_space=pl.ANY),
        scratch_shapes=[
            pltpu.VMEM((S, D), BF),
            pltpu.VMEM((D, D), BF),
            pltpu.VMEM((D, D), BF),
            pltpu.VMEM((D, D), BF),
            pltpu.VMEM((D, D), BF),
            pltpu.VMEM((D, F), BF),
            pltpu.VMEM((D, F), BF),
            pltpu.VMEM((F, D), BF),
            pltpu.VMEM((2 * D, D), BF),
            pltpu.VMEM((S, D), F32),
            pltpu.VMEM((H, S // 2, 128), U32),
            pltpu.VMEM((H, NQ, 8, TQ), U32),
            pltpu.VMEM((H, NM, DH, TM), F32),
            pltpu.VMEM((NQ, D, TQ), BF),
            pltpu.VMEM((NPRE, 16, TQ), F32),
            pltpu.VMEM((1, DH, 16 * NC, 128), F32),
            pltpu.VMEM((1, DH, 16 * NC, 128), F32),
            pltpu.VMEM((1, NQ, NJ, DH, 8, 128), F32),
            pltpu.VMEM((1, NQ, NJ, DH, 8, 128), F32),
            pltpu.VMEM((NC, TK, TQ), F32),
            pltpu.VMEM((H, NQ, TQ), F32),
            pltpu.VMEM((NM, 8, TM), F32),
            pltpu.SemaphoreType.DMA((7,)),
        ],
        compiler_params=pltpu.CompilerParams(vmem_limit_bytes=100 * 1024 * 1024,
                                             internal_scratch_in_bytes=64 * 1024),
    )(A_x.reshape(S, D), A_wqkv, A_wo, B_w_gate, B_w_up, B_w_down)
    return out.reshape(1, S, D)
```

```python
import jax
import jax.numpy as jnp
from jax import lax
import jax.experimental.pallas as pl
import jax.experimental.pallas.tpu as pltpu

S, D, H, DH, F = 2048, 512, 32, 16, 1792
TQ = 512
TK = 128
TM = 512
TN = 128
NQ = S // TQ
NC = S // TK
NJ = TQ // 128
NM = S // TM
NU = TM // TN
NSTEP = NQ * NC
EPS = 1e-5
QSCALE = (DH ** -0.5) * 1.4426950408889634
L_LO = 2.0 ** -30
L_HI = 2.0 ** 60
V_HI = 2.0 ** 60
BF = jnp.bfloat16
F32 = jnp.float32
U32 = jnp.uint32

NPRE = 8
V0 = 1
AOFF = -6
MX = [(g, i) for g in range(NSTEP + 2) for i in range(7, -1 if g % NSTEP < V0 else 0, -1)]
NMX = 7 * NSTEP + V0
LAST = {g: n for n, (g, _) in enumerate(MX)}
SUB = 4
P0, PN, FREE = 3, 57, 8
PLIST = [(k, idx, sub) for idx in range(16) for sub in range(SUB) for k in (0, 1)]


def _ln(x):
    m = jnp.mean(x, axis=-1, keepdims=True)
    xc = x - m
    v = jnp.mean(xc * xc, axis=-1, keepdims=True)
    return (xc * lax.rsqrt(v + EPS)).astype(BF)


def _swap8(x):
    return jnp.concatenate([x[r ^ 8:(r ^ 8) + 8] for r in range(0, x.shape[0], 8)], axis=0)


def _rowsum8(l, x):
    y = jnp.sum(x.reshape(x.shape[0] // 8, 8, x.shape[1]), axis=0)
    return y if l is None else l + y


def _kernel(x_hbm, wqkv_hbm, wo_hbm, wg_hbm, wu_hbm, wd_hbm, out_hbm,
            xio, wq, wk, wv, wo, wg, wu, wd, wqvt, xres, kr, qtu, vts, ots,
            ppre, kba, kbb, qba, qbb, ss, lts, vmx, sems):
    parts = range(NU)
    nt = (((1,), (1,)), ((), ()))

    def rows_of(i, u):
        return pl.ds(pl.multiple_of(i * TM + u * TN, TN), TN)

    def x_copy(i):
        return pltpu.make_async_copy(x_hbm.at[i * TM:(i + 1) * TM, :], xio.at[i * TM:(i + 1) * TM, :],
                                     sems.at[(0, 3, 6, 6)[i]])

    def out_copy(i, u):
        return pltpu.make_async_copy(xio.at[rows_of(i, u), :], out_hbm.at[rows_of(i, u), :], sems.at[5])

    cp_wk = pltpu.make_async_copy(wqkv_hbm.at[:, D:2 * D], wk, sems.at[1])
    cp_wq = pltpu.make_async_copy(wqkv_hbm.at[:, 0:D], wq, sems.at[2])
    cp_wv = pltpu.make_async_copy(wqkv_hbm.at[:, 2 * D:3 * D], wv, sems.at[3])
    cp_late = [pltpu.make_async_copy(src, dst, sems.at[4])
               for src, dst in ((wo_hbm, wo), (wg_hbm, wg), (wu_hbm, wu), (wd_hbm, wd))]

    def k_mm(xn):
        k = jnp.dot(xn, wk[...], preferred_element_type=F32)
        return pltpu.bitcast(_swap8(k).astype(BF), U32)

    def k_store(i, u, ku):
        rk = pl.ds(pl.multiple_of((i * NU + u) * (TN // 2), TN // 2), TN // 2)
        for h in range(H):
            g, hh = divmod(h, 8)
            kg = ku[:, g * 128:(g + 1) * 128]
            kr[h, rk, :] = pltpu.roll(kg, 128 - 16 * hh, 1) if hh else kg
        kf = pltpu.bitcast(ku[0:8, 0:128], BF).astype(F32)
        rb = pl.ds(pl.multiple_of((i * NU + u) * 16, 16), 16)
        for d in range(DH):
            kba[0, d, rb, :] = jnp.broadcast_to(kf[:, d:d + 1], (16, 128))

    def q_store(i, u, qt):
        q16 = (qt * QSCALE).astype(BF)
        qtu[:, i, :, u * TN:(u + 1) * TN] = pltpu.bitcast(q16, U32).reshape(H, 8, TN)
        q0 = q16[0:DH].astype(F32)
        for d in range(DH):
            qba[0, i, u, d] = jnp.broadcast_to(q0[d:d + 1, :], (8, 128))

    def v_store(i, u, vt):
        vts[:, i, :, u * TN:(u + 1) * TN] = vt.reshape(H, DH, TN)
        vmx[i, :, u * TN:(u + 1) * TN] = jnp.max(jnp.abs(vt).reshape(D // 8, 8, TN), axis=0)

    def qkv_part(i, u, xn):
        k_store(i, u, k_mm(xn))
        qv = lax.dot_general(wqvt[...], xn, nt, preferred_element_type=F32)
        q_store(i, u, qv[0:D])
        v_store(i, u, qv[D:2 * D])

    def load_ln(i, u):
        x = xio[rows_of(i, u), :].astype(F32)
        xres[rows_of(i, u), :] = x
        return _ln(x)

    def first_phase():
        x_copy(0).start()
        cp_wk.start()
        cp_wq.start()
        cp_wv.start()
        for i in range(1, NM):
            x_copy(i).start()
        x_copy(0).wait()
        xn = [load_ln(0, u) for u in parts]
        cp_wk.wait()
        kus = [k_mm(xn[u]) for u in parts[:NU // 2]]
        cp_wq.wait()
        kus += [k_mm(xn[u]) for u in parts[NU // 2:]]
        for u in parts:
            k_store(0, u, kus[u])
        wqt = wq[...].astype(F32).T.astype(BF)
        wqvt[0:D, :] = wqt
        for u in parts:
            q_store(0, u, lax.dot_general(wqt, xn[u], nt, preferred_element_type=F32))
        cp_wv.wait()
        x_copy(1).wait()
        wvt = wv[...].astype(F32).T.astype(BF)
        wqvt[D:2 * D, :] = wvt
        for u in parts:
            v_store(0, u, lax.dot_general(wvt, xn[u], nt, preferred_element_type=F32))
        xn_next = load_ln(1, 0)
        for i in range(2, NM):
            x_copy(i).wait()
        for cp in cp_late:
            cp.start()

        def block(i, xn0):
            for u in parts:
                qkv_part(i, u, xn0 if u == 0 else load_ln(i, u))
            return load_ln(jnp.minimum(i + 1, NM - 1), 0)
        lax.fori_loop(1, NM, block, xn_next)

    def get_w(h, qb):
        return jnp.concatenate([pltpu.bitcast(qtu[h, qb], BF), jnp.zeros((128 - DH, TQ), BF)], axis=0)

    def a_dot(h, w, tiles):
        ku = jnp.concatenate([kr[h, c * 64 + i * 8:c * 64 + (i + 1) * 8, :] for c, i in tiles], axis=0)
        return jnp.exp2(jnp.dot(pltpu.bitcast(ku, BF), w, preferred_element_type=F32))

    def prep_piece(h, bufs, i, anc):
        kb_ref, qb_ref = bufs
        kind, idx, sub = PLIST[i]
        qb, j = divmod(idx, NJ)
        src = kr[h, idx * 64:idx * 64 + 8, :] if kind == 0 else qtu[h, qb, :, j * 128:(j + 1) * 128]
        if anc is not None:
            src = jnp.where(anc < 0, jnp.uint32(0), src)
        val = pltpu.bitcast(src, BF).astype(F32)
        for d in range(sub * (DH // SUB), (sub + 1) * (DH // SUB)):
            if kind == 0:
                kb_ref[0, d, idx * 16:(idx + 1) * 16, :] = jnp.broadcast_to(val[:, d:d + 1], (16, 128))
            else:
                qb_ref[0, qb, j, d] = jnp.broadcast_to(val[d:d + 1, :], (8, 128))

    def vpu_block(bufs, qb, c, j, z, anc):
        kb_ref, qb_ref = bufs
        kb = kb_ref[z, :, c * 16:(c + 1) * 16, :].reshape(DH, 2, 8, 128)
        q = qb_ref[z, qb, j]
        if anc is not None:
            q0 = jnp.maximum(q[0], jnp.minimum(q[0], anc))
            q = jnp.concatenate([q0[None], q[1:]], axis=0)
        return jnp.exp2(jnp.sum(kb * q[:, None], axis=0).reshape(16, 128))

    def head(h, l_in, rd, wr):
        zs = [lax.shift_right_logical(h + j, 16) for j in range(2 * NJ)]
        hn = jnp.minimum(h + 1, H - 1)
        pt = {MX[n]: ppre[n] for n in range(NPRE)}
        ls = {0: l_in}
        ws = {}
        hist = {}
        acc = None
        nxt, ksub, kp = NPRE, V0 * NJ, 0
        for g in range(NSTEP):
            qb, c = divmod(g, NC)
            end = LAST[g] + NPRE + 1
            byunit = {}
            for n in range(nxt, end):
                byunit.setdefault(MX[n][0] // NC, []).append(n)
            nxt = end
            for u, nl in byunit.items():
                hu = hn if u == NQ else h
                if u not in ws:
                    ws[u] = get_w(hu, u % NQ)
                p = a_dot(hu, ws[u], [(MX[n][0] % NC, MX[n][1]) for n in nl])
                ls[u] = _rowsum8(ls.get(u), p)
                for k, n in enumerate(nl):
                    hist[n] = p[k * 16:(k + 1) * 16]
                    if u == NQ:
                        ppre[n - NMX] = hist[n]
                    else:
                        pt[MX[n]] = hist[n]
            while kp < len(PLIST):
                a = NPRE + (P0 * NMX) // NSTEP + (kp * PN * NMX) // (NSTEP * len(PLIST))
                if a >= end:
                    break
                free = PLIST[kp][0] == 1 and PLIST[kp][1] >= 16 - FREE
                prep_piece(hn, wr, kp, None if free else hist[a][8:16, 0:128])
                kp += 1
            while ksub < NSTEP * NJ:
                gv, j = divmod(ksub, NJ)
                a = (ksub * 7) // NJ + V0 + AOFF
                if a >= end:
                    break
                qv, cv = divmod(gv, NC)
                if gv == V0:
                    anc = pt[(gv, 0, j - 1)][0:8] if j else None
                else:
                    anc = hist[a][0:8, j * 128:(j + 1) * 128]
                pv = vpu_block(rd, qv, cv, j, zs[ksub % len(zs)], anc)
                ls[('v', qv, j)] = _rowsum8(ls.get(('v', qv, j)), pv)
                pt[(gv, 0, j)] = pv
                ksub += 1
            if c == 0:
                if acc is None:
                    l2 = jnp.concatenate([l_in, l_in], axis=0)
                    acc = jnp.where(l2 < 0, l2, 0.0)
                else:
                    acc = jnp.where(acc > jnp.inf, acc, 0.0)
            if g >= V0:
                pt[(g, 0)] = jnp.concatenate([pt.pop((g, 0, j)) for j in range(NJ)], axis=1)
            p = _swap8(jnp.concatenate([pt.pop((g, i)) for i in range(8)], axis=0))
            v = vts[h, c // NU, :, (c % NU) * TK:(c % NU + 1) * TK]
            acc = acc + jnp.dot(v, p, preferred_element_type=F32)
            if c == NC - 1:
                lv = jnp.concatenate([ls[('v', qb, j)] for j in range(NJ)], axis=1)
                lt = jnp.sum(ls[qb] + lv, axis=0, keepdims=True)
                lts[h, qb:qb + 1, :] = lt
                ots[qb, pl.ds(pl.multiple_of(h * DH, DH), DH), :] = (acc / lt).astype(BF)
        return ls[NQ]

    def attention_fast():
        p = a_dot(0, get_w(0, 0), MX[:NPRE])
        for n in range(NPRE):
            ppre[n] = p[n * 16:(n + 1) * 16]

        def body(h, l):
            return lax.cond((h & 1) == 0,
                            lambda x: head(h, x, (kba, qba), (kbb, qbb)),
                            lambda x: head(h, x, (kbb, qbb), (kba, qba)), l)
        lax.fori_loop(0, H, body, _rowsum8(None, p))
        lt = lts[...]
        bad_l = jnp.where(jnp.logical_and(lt > L_LO, lt < L_HI), 0.0, 1.0)
        bad_v = jnp.where(vmx[...] < V_HI, 0.0, 1.0)
        return jnp.maximum(jnp.max(jnp.max(bad_l, axis=0)), jnp.max(jnp.max(bad_v, axis=0)))

    def attention_exact():
        def unit(u, _):
            h = lax.shift_right_logical(u, 2)
            qb = u & (NQ - 1)
            w = get_w(h, qb)

            def pass1(c, m):
                ku = kr[h, pl.ds(pl.multiple_of(c * 64, 64), 64), :]
                s = jnp.dot(pltpu.bitcast(ku, BF), w, preferred_element_type=F32)
                ss[c] = s
                return jnp.maximum(m, jnp.max(s.reshape(TK // 8, 8, TQ), axis=0))
            m = lax.fori_loop(0, NC, pass1, jnp.full((8, TQ), -jnp.inf, F32))
            m = jnp.max(m, axis=0, keepdims=True)

            def pass2(b, carry):
                l, acc = carry
                for cc in parts:
                    p = jnp.exp2(ss[b * NU + cc] - m)
                    l = _rowsum8(l, p)
                    acc = acc + jnp.dot(vts[h, b, :, cc * TK:(cc + 1) * TK], _swap8(p),
                                        preferred_element_type=F32)
                return l, acc
            l, acc = lax.fori_loop(0, NM, pass2, (jnp.zeros((8, TQ), F32), jnp.zeros((DH, TQ), F32)))
            lt = jnp.sum(l, axis=0, keepdims=True)
            ots[qb, pl.ds(pl.multiple_of(h * DH, DH), DH), :] = (acc / lt).astype(BF)
            return 0
        lax.fori_loop(0, H * NQ, unit, 0)

    def o_part(i, u):
        return ots[i, :, u * TN:(u + 1) * TN].T

    def post(i, o0):
        x1 = [xres[rows_of(i, u), :]
              + jnp.dot(o0 if u == 0 else o_part(i, u), wo[...], preferred_element_type=F32) for u in parts]
        xn = [_ln(x1[u]) for u in parts]
        hh = [(jnp.dot(xn[u], wg[...], preferred_element_type=F32)
               * jnp.dot(xn[u], wu[...], preferred_element_type=F32)).astype(BF) for u in parts]
        return [x1[u] + jnp.dot(hh[u], wd[...], preferred_element_type=F32) for u in parts]

    def mid_block(i, o0):
        xs = post(i, o0)
        for u in parts:
            xres[rows_of(i, u), :] = xs[u]
            qkv_part(i, u, _ln(xs[u]))
        return o_part(jnp.minimum(i + 1, NM - 1), 0)

    def last_block(i, o0):
        xs = post(i, o0)
        o_next = o_part(jnp.minimum(i + 1, NM - 1), 0)
        for u in parts:
            xio[rows_of(i, u), :] = xs[u].astype(BF)
            out_copy(i, u).start()
        return o_next

    def redo(_):
        attention_exact()
        return o_part(0, 0)

    first_phase()
    for layer in range(2):
        bad = attention_fast()
        o0 = lax.cond(bad > 0.0, redo, lambda o: o, o_part(0, 0))
        if layer == 0:
            for cp in cp_late:
                cp.wait()
        lax.fori_loop(0, NM, mid_block if layer == 0 else last_block, o0)
    for i in range(NM):
        for u in parts:
            out_copy(i, u).wait()


@jax.jit
def pallas_interleave_layers__softmax_full_mha__glu_gated_bilinear__prompt_kernel(
        A_x, A_wqkv, A_wo, B_x, B_w_gate, B_w_up, B_w_down):
    out = pl.pallas_call(
        _kernel,
        out_shape=jax.ShapeDtypeStruct((S, D), BF),
        in_specs=[pl.BlockSpec(memory_space=pl.ANY)] * 6,
        out_specs=pl.BlockSpec(memory_space=pl.ANY),
        scratch_shapes=[
            pltpu.VMEM((S, D), BF),
            pltpu.VMEM((D, D), BF),
            pltpu.VMEM((D, D), BF),
            pltpu.VMEM((D, D), BF),
            pltpu.VMEM((D, D), BF),
            pltpu.VMEM((D, F), BF),
            pltpu.VMEM((D, F), BF),
            pltpu.VMEM((F, D), BF),
            pltpu.VMEM((2 * D, D), BF),
            pltpu.VMEM((S, D), F32),
            pltpu.VMEM((H, S // 2, 128), U32),
            pltpu.VMEM((H, NQ, 8, TQ), U32),
            pltpu.VMEM((H, NM, DH, TM), F32),
            pltpu.VMEM((NQ, D, TQ), BF),
            pltpu.VMEM((NPRE, 16, TQ), F32),
            pltpu.VMEM((1, DH, 16 * NC, 128), F32),
            pltpu.VMEM((1, DH, 16 * NC, 128), F32),
            pltpu.VMEM((1, NQ, NJ, DH, 8, 128), F32),
            pltpu.VMEM((1, NQ, NJ, DH, 8, 128), F32),
            pltpu.VMEM((NC, TK, TQ), F32),
            pltpu.VMEM((H, NQ, TQ), F32),
            pltpu.VMEM((NM, 8, TM), F32),
            pltpu.SemaphoreType.DMA((7,)),
        ],
        compiler_params=pltpu.CompilerParams(vmem_limit_bytes=100 * 1024 * 1024,
                                             internal_scratch_in_bytes=64 * 1024),
    )(A_x.reshape(S, D), A_wqkv, A_wo, B_w_gate, B_w_up, B_w_down)
    return out.reshape(1, S, D)
```

```python
import jax
import jax.numpy as jnp
from jax import lax
import jax.experimental.pallas as pl
import jax.experimental.pallas.tpu as pltpu

S, D, H, DH, F = 2048, 512, 32, 16, 1792
TQ = 512
TK = 128
TM = 512
TN = 128
NQ = S // TQ
NC = S // TK
NJ = TQ // 128
NM = S // TM
NU = TM // TN
NSTEP = NQ * NC
EPS = 1e-5
QSCALE = (DH ** -0.5) * 1.4426950408889634
L_LO = 2.0 ** -30
L_HI = 2.0 ** 60
V_HI = 2.0 ** 60
BF = jnp.bfloat16
F32 = jnp.float32
U32 = jnp.uint32

NPRE = 8
V0 = 1
AOFF = -6
MX = [(g, i) for g in range(NSTEP + 2) for i in range(7, -1 if g % NSTEP < V0 else 0, -1)]
NMX = 7 * NSTEP + V0
LAST = {g: n for n, (g, _) in enumerate(MX)}
SUB = 4
P0, PN, FREE = 3, 57, 8
PLIST = [(k, idx, sub) for idx in range(16) for sub in range(SUB) for k in (0, 1)]


def _ln(x):
    m = jnp.mean(x, axis=-1, keepdims=True)
    xc = x - m
    v = jnp.mean(xc * xc, axis=-1, keepdims=True)
    return (xc * lax.rsqrt(v + EPS)).astype(BF)


def _swap8(x):
    return jnp.concatenate([x[r ^ 8:(r ^ 8) + 8] for r in range(0, x.shape[0], 8)], axis=0)


def _pv(v, p):
    return jnp.dot(v, p, precision=lax.Precision.DEFAULT, preferred_element_type=F32)


def _rowsum8(l, x):
    y = jnp.sum(x.reshape(x.shape[0] // 8, 8, x.shape[1]), axis=0)
    return y if l is None else l + y


def _kernel(x_hbm, wqkv_hbm, wo_hbm, wg_hbm, wu_hbm, wd_hbm, out_hbm,
            xio, wq, wk, wv, wo, wg, wu, wd, wqvt, xres, kr, qtu, vts, ots,
            ppre, kba, kbb, qba, qbb, ss, lts, vmx, sems):
    parts = range(NU)
    nt = (((1,), (1,)), ((), ()))

    def rows_of(i, u):
        return pl.ds(pl.multiple_of(i * TM + u * TN, TN), TN)

    def x_copy(i):
        return pltpu.make_async_copy(x_hbm.at[i * TM:(i + 1) * TM, :], xio.at[i * TM:(i + 1) * TM, :],
                                     sems.at[(0, 3, 6, 6)[i]])

    def out_copy(i, u):
        return pltpu.make_async_copy(xio.at[rows_of(i, u), :], out_hbm.at[rows_of(i, u), :], sems.at[5])

    cp_wk = pltpu.make_async_copy(wqkv_hbm.at[:, D:2 * D], wk, sems.at[1])
    cp_wq = pltpu.make_async_copy(wqkv_hbm.at[:, 0:D], wq, sems.at[2])
    cp_wv = pltpu.make_async_copy(wqkv_hbm.at[:, 2 * D:3 * D], wv, sems.at[3])
    cp_late = [pltpu.make_async_copy(src, dst, sems.at[4])
               for src, dst in ((wo_hbm, wo), (wg_hbm, wg), (wu_hbm, wu), (wd_hbm, wd))]

    def k_mm(xn):
        k = jnp.dot(xn, wk[...], preferred_element_type=F32)
        return pltpu.bitcast(_swap8(k).astype(BF), U32)

    def k_store(i, u, ku):
        rk = pl.ds(pl.multiple_of((i * NU + u) * (TN // 2), TN // 2), TN // 2)
        for h in range(H):
            g, hh = divmod(h, 8)
            kg = ku[:, g * 128:(g + 1) * 128]
            kr[h, rk, :] = pltpu.roll(kg, 128 - 16 * hh, 1) if hh else kg
        kf = pltpu.bitcast(ku[0:8, 0:128], BF).astype(F32)
        rb = pl.ds(pl.multiple_of((i * NU + u) * 16, 16), 16)
        for d in range(DH):
            kba[0, d, rb, :] = jnp.broadcast_to(kf[:, d:d + 1], (16, 128))

    def q_store(i, u, qt):
        q16 = (qt * QSCALE).astype(BF)
        qtu[:, i, :, u * TN:(u + 1) * TN] = pltpu.bitcast(q16, U32).reshape(H, 8, TN)
        q0 = q16[0:DH].astype(F32)
        for d in range(DH):
            qba[0, i, u, d] = jnp.broadcast_to(q0[d:d + 1, :], (8, 128))

    def v_store(i, u, vt):
        vts[:, i, :, u * TN:(u + 1) * TN] = vt.reshape(H, DH, TN)
        vmx[i, :, u * TN:(u + 1) * TN] = jnp.max(jnp.abs(vt).reshape(D // 8, 8, TN), axis=0)

    def qkv_part(i, u, xn):
        k_store(i, u, k_mm(xn))
        qv = lax.dot_general(wqvt[...], xn, nt, preferred_element_type=F32)
        q_store(i, u, qv[0:D])
        v_store(i, u, qv[D:2 * D])

    def load_ln(i, u):
        x = xio[rows_of(i, u), :].astype(F32)
        xres[rows_of(i, u), :] = x
        return _ln(x)

    def first_phase():
        x_copy(0).start()
        cp_wk.start()
        cp_wq.start()
        cp_wv.start()
        for i in range(1, NM):
            x_copy(i).start()
        x_copy(0).wait()
        xn = [load_ln(0, u) for u in parts]
        cp_wk.wait()
        kus = [k_mm(xn[u]) for u in parts[:NU // 2]]
        cp_wq.wait()
        kus += [k_mm(xn[u]) for u in parts[NU // 2:]]
        for u in parts:
            k_store(0, u, kus[u])
        wqt = wq[...].astype(F32).T.astype(BF)
        wqvt[0:D, :] = wqt
        for u in parts:
            q_store(0, u, lax.dot_general(wqt, xn[u], nt, preferred_element_type=F32))
        cp_wv.wait()
        x_copy(1).wait()
        wvt = wv[...].astype(F32).T.astype(BF)
        wqvt[D:2 * D, :] = wvt
        for u in parts:
            v_store(0, u, lax.dot_general(wvt, xn[u], nt, preferred_element_type=F32))
        xn_next = load_ln(1, 0)
        for i in range(2, NM):
            x_copy(i).wait()
        for cp in cp_late:
            cp.start()

        def block(i, xn0):
            for u in parts:
                qkv_part(i, u, xn0 if u == 0 else load_ln(i, u))
            return load_ln(jnp.minimum(i + 1, NM - 1), 0)
        lax.fori_loop(1, NM, block, xn_next)

    def get_w(h, qb):
        return jnp.concatenate([pltpu.bitcast(qtu[h, qb], BF), jnp.zeros((128 - DH, TQ), BF)], axis=0)

    def a_dot(h, w, tiles):
        ku = jnp.concatenate([kr[h, c * 64 + i * 8:c * 64 + (i + 1) * 8, :] for c, i in tiles], axis=0)
        return jnp.exp2(jnp.dot(pltpu.bitcast(ku, BF), w, preferred_element_type=F32))

    def prep_piece(h, bufs, i, anc):
        kb_ref, qb_ref = bufs
        kind, idx, sub = PLIST[i]
        qb, j = divmod(idx, NJ)
        src = kr[h, idx * 64:idx * 64 + 8, :] if kind == 0 else qtu[h, qb, :, j * 128:(j + 1) * 128]
        if anc is not None:
            src = jnp.where(anc < 0, jnp.uint32(0), src)
        val = pltpu.bitcast(src, BF).astype(F32)
        for d in range(sub * (DH // SUB), (sub + 1) * (DH // SUB)):
            if kind == 0:
                kb_ref[0, d, idx * 16:(idx + 1) * 16, :] = jnp.broadcast_to(val[:, d:d + 1], (16, 128))
            else:
                qb_ref[0, qb, j, d] = jnp.broadcast_to(val[d:d + 1, :], (8, 128))

    def vpu_block(bufs, qb, c, j, z, anc):
        kb_ref, qb_ref = bufs
        kb = kb_ref[z, :, c * 16:(c + 1) * 16, :].reshape(DH, 2, 8, 128)
        q = qb_ref[z, qb, j]
        if anc is not None:
            q0 = jnp.maximum(q[0], jnp.minimum(q[0], anc))
            q = jnp.concatenate([q0[None], q[1:]], axis=0)
        return jnp.exp2(jnp.sum(kb * q[:, None], axis=0).reshape(16, 128))

    def head(h, l_in, rd, wr):
        zs = [lax.shift_right_logical(h + j, 16) for j in range(2 * NJ)]
        hn = jnp.minimum(h + 1, H - 1)
        pt = {MX[n]: ppre[n] for n in range(NPRE)}
        ls = {0: l_in}
        ws = {}
        hist = {}
        acc = None
        nxt, ksub, kp = NPRE, V0 * NJ, 0
        for g in range(NSTEP):
            qb, c = divmod(g, NC)
            end = LAST[g] + NPRE + 1
            byunit = {}
            for n in range(nxt, end):
                byunit.setdefault(MX[n][0] // NC, []).append(n)
            nxt = end
            for u, nl in byunit.items():
                hu = hn if u == NQ else h
                if u not in ws:
                    ws[u] = get_w(hu, u % NQ)
                p = a_dot(hu, ws[u], [(MX[n][0] % NC, MX[n][1]) for n in nl])
                ls[u] = _rowsum8(ls.get(u), p)
                for k, n in enumerate(nl):
                    hist[n] = p[k * 16:(k + 1) * 16]
                    if u == NQ:
                        ppre[n - NMX] = hist[n]
                    else:
                        pt[MX[n]] = hist[n]
            while kp < len(PLIST):
                a = NPRE + (P0 * NMX) // NSTEP + (kp * PN * NMX) // (NSTEP * len(PLIST))
                if a >= end:
                    break
                free = PLIST[kp][0] == 1 and PLIST[kp][1] >= 16 - FREE
                prep_piece(hn, wr, kp, None if free else hist[a][8:16, 0:128])
                kp += 1
            while ksub < NSTEP * NJ:
                gv, j = divmod(ksub, NJ)
                a = (ksub * 7) // NJ + V0 + AOFF
                if a >= end:
                    break
                qv, cv = divmod(gv, NC)
                if gv == V0:
                    anc = pt[(gv, 0, j - 1)][0:8] if j else None
                else:
                    anc = hist[a][0:8, j * 128:(j + 1) * 128]
                pv = vpu_block(rd, qv, cv, j, zs[ksub % len(zs)], anc)
                ls[('v', qv, j)] = _rowsum8(ls.get(('v', qv, j)), pv)
                pt[(gv, 0, j)] = pv
                ksub += 1
            if c == 0:
                if acc is None:
                    l2 = jnp.concatenate([l_in, l_in], axis=0)
                    acc = jnp.where(l2 < 0, l2, 0.0)
                else:
                    acc = jnp.where(acc > jnp.inf, acc, 0.0)
            if g >= V0:
                pt[(g, 0)] = jnp.concatenate([pt.pop((g, 0, j)) for j in range(NJ)], axis=1)
            p = _swap8(jnp.concatenate([pt.pop((g, i)) for i in range(8)], axis=0))
            v = vts[h, c // NU, :, (c % NU) * TK:(c % NU + 1) * TK]
            acc = acc + _pv(v, p)
            if c == NC - 1:
                lv = jnp.concatenate([ls[('v', qb, j)] for j in range(NJ)], axis=1)
                lt = jnp.sum(ls[qb] + lv, axis=0, keepdims=True)
                lts[h, qb:qb + 1, :] = lt
                ots[qb, pl.ds(pl.multiple_of(h * DH, DH), DH), :] = (acc / lt).astype(BF)
        assert kp == len(PLIST) and ksub == NSTEP * NJ and not pt
        return ls[NQ]

    def attention_fast():
        p = a_dot(0, get_w(0, 0), MX[:NPRE])
        for n in range(NPRE):
            ppre[n] = p[n * 16:(n + 1) * 16]

        def body(h, l):
            return lax.cond((h & 1) == 0,
                            lambda x: head(h, x, (kba, qba), (kbb, qbb)),
                            lambda x: head(h, x, (kbb, qbb), (kba, qba)), l)
        lax.fori_loop(0, H, body, _rowsum8(None, p))
        lt = lts[...]
        bad_l = jnp.where(jnp.logical_and(lt > L_LO, lt < L_HI), 0.0, 1.0)
        bad_v = jnp.where(vmx[...] < V_HI, 0.0, 1.0)
        return jnp.maximum(jnp.max(jnp.max(bad_l, axis=0)), jnp.max(jnp.max(bad_v, axis=0)))

    def attention_exact():
        def unit(u, _):
            h = lax.shift_right_logical(u, 2)
            qb = u & (NQ - 1)
            w = get_w(h, qb)

            def pass1(c, m):
                ku = kr[h, pl.ds(pl.multiple_of(c * 64, 64), 64), :]
                s = jnp.dot(pltpu.bitcast(ku, BF), w, preferred_element_type=F32)
                ss[c] = s
                return jnp.maximum(m, jnp.max(s.reshape(TK // 8, 8, TQ), axis=0))
            m = lax.fori_loop(0, NC, pass1, jnp.full((8, TQ), -jnp.inf, F32))
            m = jnp.max(m, axis=0, keepdims=True)

            def pass2(b, carry):
                l, acc = carry
                for cc in parts:
                    p = jnp.exp2(ss[b * NU + cc] - m)
                    l = _rowsum8(l, p)
                    acc = acc + _pv(vts[h, b, :, cc * TK:(cc + 1) * TK], _swap8(p))
                return l, acc
            l, acc = lax.fori_loop(0, NM, pass2, (jnp.zeros((8, TQ), F32), jnp.zeros((DH, TQ), F32)))
            lt = jnp.sum(l, axis=0, keepdims=True)
            ots[qb, pl.ds(pl.multiple_of(h * DH, DH), DH), :] = (acc / lt).astype(BF)
            return 0
        lax.fori_loop(0, H * NQ, unit, 0)

    def o_part(i, u):
        return ots[i, :, u * TN:(u + 1) * TN].T

    def post(i, o0):
        x1 = [xres[rows_of(i, u), :]
              + jnp.dot(o0 if u == 0 else o_part(i, u), wo[...], preferred_element_type=F32) for u in parts]
        xn = [_ln(x1[u]) for u in parts]
        hh = [(jnp.dot(xn[u], wg[...], preferred_element_type=F32)
               * jnp.dot(xn[u], wu[...], preferred_element_type=F32)).astype(BF) for u in parts]
        return [x1[u] + jnp.dot(hh[u], wd[...], preferred_element_type=F32) for u in parts]

    def mid_block(i, o0):
        xs = post(i, o0)
        for u in parts:
            xres[rows_of(i, u), :] = xs[u]
            qkv_part(i, u, _ln(xs[u]))
        return o_part(jnp.minimum(i + 1, NM - 1), 0)

    def last_block(i, o0):
        xs = post(i, o0)
        o_next = o_part(jnp.minimum(i + 1, NM - 1), 0)
        for u in parts:
            xio[rows_of(i, u), :] = xs[u].astype(BF)
            out_copy(i, u).start()
        return o_next

    def redo(_):
        attention_exact()
        return o_part(0, 0)

    first_phase()
    for layer in range(2):
        bad = attention_fast()
        o0 = lax.cond(bad > 0.0, redo, lambda o: o, o_part(0, 0))
        if layer == 0:
            for cp in cp_late:
                cp.wait()
        lax.fori_loop(0, NM, mid_block if layer == 0 else last_block, o0)
    for i in range(NM):
        for u in parts:
            out_copy(i, u).wait()


@jax.jit
def pallas_interleave_layers__softmax_full_mha__glu_gated_bilinear__prompt_kernel(
        A_x, A_wqkv, A_wo, B_x, B_w_gate, B_w_up, B_w_down):
    out = pl.pallas_call(
        _kernel,
        out_shape=jax.ShapeDtypeStruct((S, D), BF),
        in_specs=[pl.BlockSpec(memory_space=pl.ANY)] * 6,
        out_specs=pl.BlockSpec(memory_space=pl.ANY),
        scratch_shapes=[
            pltpu.VMEM((S, D), BF),
            pltpu.VMEM((D, D), BF),
            pltpu.VMEM((D, D), BF),
            pltpu.VMEM((D, D), BF),
            pltpu.VMEM((D, D), BF),
            pltpu.VMEM((D, F), BF),
            pltpu.VMEM((D, F), BF),
            pltpu.VMEM((F, D), BF),
            pltpu.VMEM((2 * D, D), BF),
            pltpu.VMEM((S, D), F32),
            pltpu.VMEM((H, S // 2, 128), U32),
            pltpu.VMEM((H, NQ, 8, TQ), U32),
            pltpu.VMEM((H, NM, DH, TM), F32),
            pltpu.VMEM((NQ, D, TQ), BF),
            pltpu.VMEM((NPRE, 16, TQ), F32),
            pltpu.VMEM((1, DH, 16 * NC, 128), F32),
            pltpu.VMEM((1, DH, 16 * NC, 128), F32),
            pltpu.VMEM((1, NQ, NJ, DH, 8, 128), F32),
            pltpu.VMEM((1, NQ, NJ, DH, 8, 128), F32),
            pltpu.VMEM((NC, TK, TQ), F32),
            pltpu.VMEM((H, NQ, TQ), F32),
            pltpu.VMEM((NM, 8, TM), F32),
            pltpu.SemaphoreType.DMA((7,)),
        ],
        compiler_params=pltpu.CompilerParams(vmem_limit_bytes=100 * 1024 * 1024,
                                             internal_scratch_in_bytes=64 * 1024),
    )(A_x.reshape(S, D), A_wqkv, A_wo, B_w_gate, B_w_up, B_w_down)
    return out.reshape(1, S, D)
```
